```python
import jax
import jax.numpy as jnp

def _softmax(x, axis=-1):
    return jax.nn.softmax(x, axis=axis)
def _gelu(x):
    return jax.nn.gelu(x, approximate=True)
def _silu(x):
    return jax.nn.silu(x)
def _sigmoid(x):
    return jax.nn.sigmoid(x)
def _layernorm(x, axis=-1, eps=1e-5):
    m = jnp.mean(x, axis=axis, keepdims=True)
    v = jnp.var(x, axis=axis, keepdims=True)
    return (x - m) / jnp.sqrt(v + eps)
def _scatter_add(tgt, idx, src, axis=0):
    return tgt.at[idx].add(src)
def _segment_sum(src, seg, n):
    return jax.ops.segment_sum(src, seg, n)
class _Rng:
    def __init__(self, key):
        self._k = key
    def _next(self):
        self._k, sub = jax.random.split(self._k)
        return sub
    def normal(self, shape):
        return jax.random.normal(self._next(), shape, dtype=jnp.bfloat16)
    def randint(self, lo, hi, shape):
        return jax.random.randint(self._next(), shape, lo, hi, dtype=jnp.int32)
    def uniform(self, shape, lo=0.0, hi=1.0):
        return jax.random.uniform(self._next(), shape, jnp.bfloat16, lo, hi)
    def permutation(self, n):
        return jax.random.permutation(self._next(), n)


kernel_name = 'recurrent_scan__mha_block_cached__moe_arch_mod__decode'

def setup_inputs():
    _rng = _Rng(jax.random.key(int.from_bytes(__import__("os").urandom(4), "little")))
    _w = (lambda a: (lambda t: t.astype(jnp.bfloat16) if jnp.issubdtype(t.dtype, jnp.floating) else t)(jnp.asarray(a)))
    def _A_setup():
        B, Sq, D = 2, 1, 512
        H, Sk, Dh = 32, 16384, 128
        return {
            "x": _w((lambda *s: _rng.normal(s) * 0.05)(B, Sq, D)),
            "k_cache": _w((lambda *s: _rng.normal(s) * 0.05)(B, H, Sk, Dh)),
            "v_cache": _w((lambda *s: _rng.normal(s) * 0.05)(B, H, Sk, Dh)),
            "wq": _w((lambda *s: _rng.normal(s) * 0.05)(D, H * Dh) * (D ** -0.5)),
            "wo": _w((lambda *s: _rng.normal(s) * 0.05)(H * Dh, D) * ((H * Dh) ** -0.5)),
        }
    _A_in = _A_setup()

    def _B_setup():
        B, S, D, F, C = 2, 1, 512, 1792, 1
        return {
            "x": _w((lambda *s: _rng.normal(s) * 0.05)(B, S, D)),
            "w_r": _w((lambda *s: _rng.normal(s) * 0.05)(D)),
            "w_gate": _w((lambda *s: _rng.normal(s) * 0.05)(D, F)),
            "w_up": _w((lambda *s: _rng.normal(s) * 0.05)(D, F)),
            "w_down": _w((lambda *s: _rng.normal(s) * 0.05)(F, D)),
        }
    _B_in = _B_setup()

    return {
        "A_x": _A_in["x"],
        "A_k_cache": _A_in["k_cache"],
        "A_v_cache": _A_in["v_cache"],
        "A_wq": _A_in["wq"],
        "A_wo": _A_in["wo"],
        "B_x": _B_in["x"],
        "B_w_r": _B_in["w_r"],
        "B_w_gate": _B_in["w_gate"],
        "B_w_up": _B_in["w_up"],
        "B_w_down": _B_in["w_down"],
    }

def reference(A_x, A_k_cache, A_v_cache, A_wq, A_wo, B_x, B_w_r, B_w_gate, B_w_up, B_w_down):
    def _A_ref(x, k_cache, v_cache, wq, wo):
        B, Sq, D = x.shape
        H, Dh = 32, 128
        q = (lambda x, *d: x.transpose(*d))((x @ wq).reshape(B, Sq, H, Dh), 0, 2, 1, 3)
        scores = jnp.einsum("bhqd,bhkd->bhqk", q, k_cache) * (Dh ** -0.5)
        p = _softmax(scores, axis=-1)
        o = jnp.einsum("bhqk,bhkd->bhqd", p, v_cache)
        return (lambda x, *d: x.transpose(*d))(o, 0, 2, 1, 3).reshape(B, Sq, H * Dh) @ wo

    def _B_ref(x, w_r, w_gate, w_up, w_down):
        B, S, D = x.shape
        C = 1
        r = x @ w_r
        idx = jnp.argsort(-r, axis=-1)[:, :C]
        idx_e = jnp.repeat(idx.reshape(B, C, 1), D, axis=2)
        x_sel = jnp.take_along_axis(x, idx_e, axis=1)
        g = _silu(x_sel @ w_gate)
        u = x_sel @ w_up
        y = (g * u) @ w_down
        r_sel = _sigmoid(jnp.take_along_axis(r, idx, axis=1))
        y = y * r_sel.reshape(B, C, 1)
        b_off = (jnp.arange(B) * S).reshape(B, 1)
        flat_idx = (idx + b_off).reshape(B * C)
        zero = (x * 0.0).reshape(B * S, D)
        upd = _scatter_add(zero, flat_idx, y.reshape(B * C, D), axis=0)
        return x + upd.reshape(B, S, D)

    x = A_x
    xn = _layernorm(x, axis=-1)
    s = _A_ref(xn, A_k_cache, A_v_cache, A_wq, A_wo)
    g = _silu(_B_ref(xn, B_w_r, B_w_gate, B_w_up, B_w_down))
    return x + s * g
```

```python
import functools
import numpy as np
import jax
import jax.numpy as jnp
from jax.experimental import pallas as pl
from jax.experimental.pallas import tpu as pltpu

T = 128


def build(G=8, NS=8, MR=8, bounds=False):
    B, D, H, Sk, Dh, F = 2, 512, 32, 16384, 128, 1792
    BLK = G * T
    NPER = Sk // BLK
    NSTEP = B * H * NPER
    bf = jnp.bfloat16
    f32 = jnp.float32
    LOG2E = 1.4426950408889634
    CEXP = float(Dh ** -0.5 * LOG2E)
    NEG = float(np.finfo(np.float32).min)

    def kern(x_hbm, wr_hbm, k_hbm, v_hbm, wq_hbm, wo_hbm, wg_hbm, wu_hbm, wd_hbm,
             o_ref,
             xb, wrb, kb, vb, wqb, wob, wgb, wub, wdb, ob, ks, vs, ws):
        def kv_start(step, slot):
            h = step // (B * NPER)
            b = (step // NPER) % B
            c = step % NPER
            base = (b * H + h) * Sk + c * BLK
            for j in range(G):
                st = pl.multiple_of(base + j * T, T)
                pltpu.make_async_copy(k_hbm.at[pl.ds(st, T)], kb.at[slot, pl.ds(j * T, T)], ks.at[slot]).start(priority=0)
                pltpu.make_async_copy(v_hbm.at[pl.ds(st, T)], vb.at[slot, pl.ds(j * T, T)], vs.at[slot]).start(priority=1)

        def pieces(src, dst, sem, r, c):
            out = []
            for i in range(0, src.shape[0], r):
                for j in range(0, src.shape[1], c):
                    out.append(pltpu.make_async_copy(src.at[pl.ds(i, r), pl.ds(j, c)], dst.at[pl.ds(i, r), pl.ds(j, c)], sem))
            return out

        def start_all(cps):
            for n, cp in enumerate(cps):
                cp.start(priority=n % 2)

        def wait_full(buf, sem):
            pltpu.make_async_copy(buf, buf, sem).wait()

        cx = pltpu.make_async_copy(x_hbm, xb, ws.at[0])
        cr = pltpu.make_async_copy(wr_hbm, wrb, ws.at[1])
        cx.start(priority=0)
        cr.start(priority=1)
        start_all(pieces(wg_hbm, wgb, ws.at[2], 16, 896))
        start_all(pieces(wu_hbm, wub, ws.at[3], 16, 896))
        start_all(pieces(wd_hbm, wdb, ws.at[4], 32, 512))
        start_all(pieces(wq_hbm, wqb, ws.at[5], 16, 1024))
        cx.wait()
        cr.wait()
        x = xb[...].astype(f32)
        if MR != B:
            x = jnp.concatenate([x, jnp.zeros((MR - B, D), f32)], axis=0)
        mu = jnp.mean(x, axis=-1, keepdims=True)
        xc = x - mu
        var = jnp.mean(xc * xc, axis=-1, keepdims=True)
        xn = xc / jnp.sqrt(var + 1e-5)
        xnb = xn.astype(bf)
        xn = xnb.astype(f32)
        for s in range(NS - 1):
            kv_start(s, s)
        wait_full(wgb, ws.at[2]); wait_full(wub, ws.at[3]); wait_full(wdb, ws.at[4])
        wr = wrb[...].astype(f32)
        r = 0.0
        for j in range(D // 128):
            r = r + xn[:, j * 128:(j + 1) * 128] * wr[j:j + 1, :]
        r = jnp.sum(r, axis=-1, keepdims=True)
        gt = jnp.dot(xnb, wgb[...], preferred_element_type=f32)
        up = jnp.dot(xnb, wub[...], preferred_element_type=f32)
        hh = (gt * jax.nn.sigmoid(gt) * up).astype(bf)
        y = jnp.dot(hh, wdb[...], preferred_element_type=f32)
        y = y * jax.nn.sigmoid(r)
        z = xn + (xn * 0.0 + y)
        gate = z * jax.nn.sigmoid(z)
        wait_full(wqb, ws.at[5])

        rows = jax.lax.broadcasted_iota(jnp.int32, (MR, Dh), 0)

        def head(h, carry):
            hoff = pl.multiple_of(h * Dh, Dh)
            q = jnp.dot(xnb, wqb[:, pl.ds(hoff, Dh)], preferred_element_type=f32).astype(bf)

            def batch(b, o):
                def step(c, st):
                    m, l, acc = st
                    i = (h * B + b) * NPER + c
                    slot = i % NS

                    @pl.when(i + NS - 1 < NSTEP)
                    def _():
                        kv_start(i + NS - 1, (i + NS - 1) % NS)

                    wait_full(kb.at[slot], ks.at[slot])
                    wait_full(vb.at[slot], vs.at[slot])
                    s = jax.lax.dot_general(q, kb[slot], (((1,), (1,)), ((), ())), preferred_element_type=f32)
                    m_new = jnp.maximum(m, jnp.max(s, axis=-1, keepdims=True))
                    alpha = jnp.exp2((m - m_new) * CEXP)
                    p = jnp.exp2((s - m_new) * CEXP)
                    ps = p[:, 0:128]
                    for j in range(1, G):
                        ps = ps + p[:, j * 128:(j + 1) * 128]
                    l = alpha * l + ps
                    acc = alpha * acc + jnp.dot(p.astype(bf), vb[slot], preferred_element_type=f32)
                    return m_new, l, acc
                init = (jnp.full((MR, 1), NEG, f32), jnp.zeros((MR, 128), f32), jnp.zeros((MR, Dh), f32))
                m, l, acc = jax.lax.fori_loop(0, NPER, step, init)
                ob_ = acc / jnp.sum(l, axis=-1, keepdims=True)
                return jnp.where(rows == b, ob_, o)
            o = jax.lax.fori_loop(0, B, batch, jnp.zeros((MR, Dh), f32))
            ob[:, pl.ds(hoff, Dh)] = o
            return carry

        jax.lax.fori_loop(0, H, head, 0)
        start_all(pieces(wo_hbm, wob, ws.at[6], 32, 512))
        wait_full(wob, ws.at[6])
        sa = jnp.dot(ob[...].astype(bf), wob[...], preferred_element_type=f32)
        res = x + sa * gate
        o_ref[...] = res[:B].astype(o_ref.dtype)

    def fn(A_x, A_k, A_v, wq, wo, B_x, wr, wg, wu, wd):
        hbm = pl.BlockSpec(memory_space=pltpu.HBM)
        out = pl.pallas_call(
            kern,
            out_shape=jax.ShapeDtypeStruct((B, D), A_x.dtype),
            in_specs=[hbm] * 9,
            out_specs=pl.BlockSpec(memory_space=pltpu.VMEM),
            scratch_shapes=[
                pltpu.VMEM((B, D), bf), pltpu.VMEM((D // 128, 128), bf),
                pltpu.VMEM((NS, BLK, Dh), bf), pltpu.VMEM((NS, BLK, Dh), bf),
                pltpu.VMEM((D, H * Dh), bf), pltpu.VMEM((H * Dh, D), bf),
                pltpu.VMEM((D, F), bf), pltpu.VMEM((D, F), bf), pltpu.VMEM((F, D), bf),
                pltpu.VMEM((MR, H * Dh), f32),
                pltpu.SemaphoreType.DMA((NS,)), pltpu.SemaphoreType.DMA((NS,)), pltpu.SemaphoreType.DMA((8,)),
            ],
            compiler_params=pltpu.CompilerParams(vmem_limit_bytes=100 * 1024 * 1024, disable_bounds_checks=not bounds),
        )(A_x.reshape(B, D), wr.reshape(D // 128, 128), A_k.reshape(B * H * Sk, Dh), A_v.reshape(B * H * Sk, Dh), wq, wo, wg, wu, wd)
        return out.reshape(B, 1, D)
    return fn


_impl = build(G=16, NS=8, MR=8)


@jax.jit
def pallas_recurrent_scan__mha_block_cached__moe_arch_mod__decode_kernel(
    A_x, A_k_cache, A_v_cache, A_wq, A_wo, B_x, B_w_r, B_w_gate, B_w_up, B_w_down
):
    return _impl(A_x, A_k_cache, A_v_cache, A_wq, A_wo, B_x, B_w_r, B_w_gate, B_w_up, B_w_down)
```

```python
import numpy as np
import jax
import jax.numpy as jnp
from jax import lax
from jax.experimental import pallas as pl
from jax.experimental.pallas import tpu as pltpu

B, D, H, SK, DH, F = 2, 512, 32, 16384, 128, 1792
R = B * H * SK
MR = 8

BLK = 2048
PC = 192
GP = 8
RP = 64
NG = RP // GP
NPER = SK // BLK
NSTEP = R // BLK
NFULL = R // PC

FC = 256
NFC = F // FC
LAP = 7 * NFC

WW = 4 * DH
NWO = H * DH // WW
WP = 32
NWP = H * DH // (2 * WP)
WO_PER_STEP = 16

TAIL = min(i for i in range(NSTEP) if 32 * ((i + 1) // 3) + 11 * ((i + 1) % 3) + LAP >= NFULL)
assert LAP <= 52 and (NSTEP - TAIL) * WO_PER_STEP >= NWP

EXP_SCALE = float(DH ** -0.5 * np.log2(np.e))
F32_MIN = float(np.finfo(np.float32).min)


def _ds(start, size, multiple):
    return pl.ds(start if isinstance(start, int) else pl.multiple_of(start, multiple), size)


def _wait_full(buf, sem):
    pltpu.make_async_copy(buf, buf, sem).wait()


def _kernel(x_hbm, wr_hbm, k_hbm, v_hbm, wq_hbm, wo_hbm, wg_hbm, wu_hbm, wd_hbm,
            out_ref,
            xb, wrb, kb, vb, wqb, wob, wgb, wub, wdb, ob, ksem, vsem, wsem, osem):
    bf16, f32 = jnp.bfloat16, jnp.float32

    def kv_piece(src, buf, sem, p, n=PC):
        return pltpu.make_async_copy(
            src.at[_ds(p * PC, n, 64)],
            buf.at[_ds((p & (RP - 1)) * PC, n, 64)],
            sem.at[(p >> 3) & (NG - 1)])

    def kv_pair(p, carry):
        kv_piece(v_hbm, vb, vsem, p).start(priority=1)
        kv_piece(k_hbm, kb, ksem, p - 1).start(priority=0)
        return carry

    def kv_wait_group(g, n=GP * PC):
        slot = g & (NG - 1)
        rows = _ds(slot * (GP * PC), n, GP * PC)
        _wait_full(kb.at[rows], ksem.at[slot])
        _wait_full(vb.at[rows], vsem.at[slot])

    def w_piece(src, dst, sem, *idx):
        return pltpu.make_async_copy(src.at[idx], dst.at[idx], sem)

    def gate_up_pair(j, carry):
        rows = _ds(j * 8, 8, 8)
        w_piece(wg_hbm, wgb, wsem.at[2], rows).start(priority=1)
        w_piece(wu_hbm, wub, wsem.at[3], rows).start(priority=0)
        return carry

    def down_pair(j, carry):
        w_piece(wd_hbm, wdb, wsem.at[4], _ds(j * 32, 32, 32)).start(priority=1)
        w_piece(wd_hbm, wdb, wsem.at[4], _ds(F // 2 + j * 32, 32, 32)).start(priority=0)
        return carry

    def wq_pair(j, carry):
        cols = _ds((j & 1) * 2048, 2048, 2048)
        w_piece(wq_hbm, wqb, wsem.at[5], _ds((j >> 1) * 8, 8, 8), cols).start(priority=1)
        w_piece(wq_hbm, wqb, wsem.at[5], _ds(D // 2 + (j >> 1) * 8, 8, 8), cols).start(priority=0)
        return carry

    def wo_pair(j, carry):
        sem = osem.at[lax.div(j, WW // (2 * WP))]
        w_piece(wo_hbm, wob, sem, _ds(j * (2 * WP), WP, WP)).start(priority=1)
        w_piece(wo_hbm, wob, sem, _ds(j * (2 * WP) + WP, WP, WP)).start(priority=0)
        return carry

    x_copy = pltpu.make_async_copy(x_hbm, xb, wsem.at[0])
    wr_copy = pltpu.make_async_copy(wr_hbm, wrb, wsem.at[1])
    lax.fori_loop(0, D // 8, gate_up_pair, 0)
    x_copy.start(priority=1)
    wr_copy.start(priority=0)
    lax.fori_loop(0, F // 64, down_pair, 0)
    lax.fori_loop(0, D // 8, wq_pair, 0)
    kv_piece(v_hbm, vb, vsem, 0).start(priority=1)
    x_copy.wait()
    wr_copy.wait()

    x = jnp.concatenate([xb[...].astype(f32), jnp.zeros((MR - B, D), f32)], axis=0)
    xc = x - jnp.mean(x, axis=-1, keepdims=True)
    var = jnp.mean(xc * xc, axis=-1, keepdims=True)
    xn16 = (xc / jnp.sqrt(var + 1e-5)).astype(bf16)
    xn = xn16.astype(f32)

    wr = wrb[...].astype(f32)
    r = xn[:, 0:128] * wr[0:1, :]
    for j in range(1, D // 128):
        r = r + xn[:, j * 128:(j + 1) * 128] * wr[j:j + 1, :]
    r = jnp.sum(r, axis=-1, keepdims=True)

    _wait_full(wgb, wsem.at[2])
    _wait_full(wub, wsem.at[3])
    _wait_full(wdb, wsem.at[4])

    def ffn_chunk(f, y):
        lax.fori_loop(jnp.maximum(f * 7, 1), f * 7 + 7, kv_pair, 0)
        cols = _ds(f * FC, FC, FC)
        g = jnp.dot(xn16, wgb[:, cols], preferred_element_type=f32)
        u = jnp.dot(xn16, wub[:, cols], preferred_element_type=f32)
        hidden = (g * jax.nn.sigmoid(g) * u).astype(bf16)
        return y + jnp.dot(hidden, wdb[cols, :], preferred_element_type=f32)

    y = lax.fori_loop(0, NFC, ffn_chunk, jnp.zeros((MR, D), f32))
    z = xn + (xn * 0.0 + y * jax.nn.sigmoid(r))
    gate = z * jax.nn.sigmoid(z)

    _wait_full(wqb, wsem.at[5])

    def head(bh, carry):
        cols = _ds((bh & (H - 1)) * DH, DH, DH)
        q = jnp.dot(xn16, wqb[:, cols], preferred_element_type=f32).astype(bf16)

        def step(c, state):
            i = bh * NPER + c
            sup = lax.div(i, 3)
            t = i - 3 * sup
            p0 = 32 * sup + 11 * t + LAP
            p1 = p0 + jnp.where(t == 2, 10, 11)
            lax.fori_loop(p0, jnp.minimum(p1, NFULL), kv_pair, 0)

            @pl.when(i >= TAIL)
            def _():
                @pl.when(i == TAIL)
                def _():
                    kv_piece(v_hbm, vb, vsem, NFULL, R - NFULL * PC).start(priority=1)
                    kv_piece(k_hbm, kb, ksem, NFULL - 1).start(priority=0)
                    kv_piece(k_hbm, kb, ksem, NFULL, R - NFULL * PC).start(priority=0)

                w0 = (i - TAIL) * WO_PER_STEP
                lax.fori_loop(jnp.minimum(w0, NWP), jnp.minimum(w0 + WO_PER_STEP, NWP), wo_pair, 0)

            @pl.when(t == 0)
            def _():
                kv_wait_group(4 * sup)

            @pl.when(i < NSTEP - 1)
            def _():
                kv_wait_group(4 * sup + t + 1)

            @pl.when(i == NSTEP - 1)
            def _():
                last = NFULL // GP
                kv_wait_group(last, R - last * GP * PC)

            m, l, acc = state
            rows = _ds(((sup & 1) * 3 + t) * BLK, BLK, BLK)
            s = lax.dot_general(q, kb[rows, :], (((1,), (1,)), ((), ())),
                                preferred_element_type=f32)
            m_new = jnp.maximum(m, jnp.max(s, axis=-1, keepdims=True))
            alpha = jnp.exp2((m - m_new) * EXP_SCALE)
            p = jnp.exp2((s - m_new) * EXP_SCALE)
            p_sum = p[:, 0:128]
            for j in range(1, BLK // 128):
                p_sum = p_sum + p[:, j * 128:(j + 1) * 128]
            l = alpha * l + p_sum
            acc = alpha * acc + jnp.dot(p.astype(bf16), vb[rows, :], preferred_element_type=f32)
            return m_new, l, acc

        init = (jnp.full((MR, 1), F32_MIN, f32), jnp.zeros((MR, 128), f32),
                jnp.zeros((MR, DH), f32))
        _, l, acc = lax.fori_loop(0, NPER, step, init)
        ob[lax.div(bh, H), :, cols] = acc / jnp.sum(l, axis=-1, keepdims=True)
        return carry

    lax.fori_loop(0, B * H, head, 0)

    first_row = lax.broadcasted_iota(jnp.int32, (MR, WW), 0) == 0

    def project(c, attn):
        sl = _ds(c * WW, WW, WW)
        o = jnp.where(first_row, ob[0, :, sl], ob[1, :, sl]).astype(bf16)
        _wait_full(wob.at[sl], osem.at[c])
        return attn + jnp.dot(o, wob[sl, :], preferred_element_type=f32)

    attn = lax.fori_loop(0, NWO, project, jnp.zeros((MR, D), f32))
    out_ref[...] = (x + attn * gate)[:B].astype(out_ref.dtype)


@jax.jit
def pallas_recurrent_scan__mha_block_cached__moe_arch_mod__decode_kernel(
    A_x: jax.Array,
    A_k_cache: jax.Array,
    A_v_cache: jax.Array,
    A_wq: jax.Array,
    A_wo: jax.Array,
    B_x: jax.Array,
    B_w_r: jax.Array,
    B_w_gate: jax.Array,
    B_w_up: jax.Array,
    B_w_down: jax.Array,
):
    del B_x
    assert A_x.shape == (B, 1, D) and A_k_cache.shape == A_v_cache.shape == (B, H, SK, DH)
    assert B_w_gate.shape == (D, F)
    bf16 = jnp.bfloat16
    out = pl.pallas_call(
        _kernel,
        out_shape=jax.ShapeDtypeStruct((B, D), A_x.dtype),
        in_specs=[pl.BlockSpec(memory_space=pltpu.HBM)] * 9,
        out_specs=pl.BlockSpec(memory_space=pltpu.VMEM),
        scratch_shapes=[
            pltpu.VMEM((B, D), bf16),
            pltpu.VMEM((D // 128, 128), bf16),
            pltpu.VMEM((RP * PC, DH), bf16),
            pltpu.VMEM((RP * PC, DH), bf16),
            pltpu.VMEM((D, H * DH), bf16),
            pltpu.VMEM((H * DH, D), bf16),
            pltpu.VMEM((D, F), bf16),
            pltpu.VMEM((D, F), bf16),
            pltpu.VMEM((F, D), bf16),
            pltpu.VMEM((B, MR, H * DH), jnp.float32),
            pltpu.SemaphoreType.DMA((NG,)),
            pltpu.SemaphoreType.DMA((NG,)),
            pltpu.SemaphoreType.DMA((6,)),
            pltpu.SemaphoreType.DMA((NWO,)),
        ],
        compiler_params=pltpu.CompilerParams(vmem_limit_bytes=48 * 1024 * 1024),
    )(
        A_x.reshape(B, D),
        B_w_r.reshape(D // 128, 128),
        A_k_cache.reshape(R, DH),
        A_v_cache.reshape(R, DH),
        A_wq, A_wo, B_w_gate, B_w_up, B_w_down,
    )
    return out.reshape(B, 1, D)
```
